```python
import os as _os
_os.environ.setdefault("JAX_PLATFORMS", "cpu")
import jax
import jax.numpy as jnp

def _softmax(x, axis=-1):
    return jax.nn.softmax(x, axis=axis)
def _gelu(x):
    return jax.nn.gelu(x, approximate=True)
def _silu(x):
    return jax.nn.silu(x)
def _sigmoid(x):
    return jax.nn.sigmoid(x)
def _layernorm(x, axis=-1, eps=1e-5):
    m = jnp.mean(x, axis=axis, keepdims=True)
    v = jnp.var(x, axis=axis, keepdims=True)
    return (x - m) / jnp.sqrt(v + eps)
def _scatter_add(tgt, idx, src, axis=0):
    return tgt.at[idx].add(src)
def _segment_sum(src, seg, n):
    return jax.ops.segment_sum(src, seg, n)
class _Rng:
    def __init__(self, key):
        self._k = key
    def _next(self):
        self._k, sub = jax.random.split(self._k)
        return sub
    def normal(self, shape):
        return jax.random.normal(self._next(), shape, dtype=jnp.bfloat16)
    def randint(self, lo, hi, shape):
        return jax.random.randint(self._next(), shape, lo, hi, dtype=jnp.int32)
    def uniform(self, shape, lo=0.0, hi=1.0):
        return jax.random.uniform(self._next(), shape, jnp.bfloat16, lo, hi)
    def permutation(self, n):
        return jax.random.permutation(self._next(), n)


kernel_name = 'gated_mix__ssm_conv_s5__glu_gated_geglu__prompt'

def setup_inputs():
    _rng = _Rng(jax.random.key(int.from_bytes(__import__("os").urandom(4), "little")))
    _w = (lambda a: (lambda t: t.astype(jnp.bfloat16) if jnp.issubdtype(t.dtype, jnp.floating) else t)(jnp.asarray(a)))
    def _A_setup():
        B, S, D = 1, 2048, 1024
        P = D
        Lambda_re = -0.5 * jnp.exp((lambda *s: _rng.normal(s) * 0.4)(P))
        Lambda_im = (lambda *s: _rng.normal(s) * 0.4)(P) * 1.0
        B_re = (lambda *s: _rng.normal(s) * 0.4)(P, D) * (D ** -0.5)
        B_im = (lambda *s: _rng.normal(s) * 0.4)(P, D) * (D ** -0.5)
        C_re = (lambda *s: _rng.normal(s) * 0.4)(D, P) * (P ** -0.5)
        C_im = (lambda *s: _rng.normal(s) * 0.4)(D, P) * (P ** -0.5)
        log_dt = (lambda *s: _rng.normal(s) * 0.4)(P) * 0.3 - 2.0
        Dskip = (lambda *s: _rng.normal(s) * 0.4)(D)
        return {
            "x": _w((lambda *s: _rng.normal(s) * 0.05)(B, S, D)),
            "Lambda_re": _w(Lambda_re),
            "Lambda_im": _w(Lambda_im),
            "B_re": _w(B_re),
            "B_im": _w(B_im),
            "C_re": _w(C_re),
            "C_im": _w(C_im),
            "log_dt": _w(log_dt),
            "Dskip": _w(Dskip),
        }
    _A_in = _A_setup()

    def _B_setup():
        B, S, Dm, Df = 1, 2048, 1024, 3584
        return {
            "x": _w((lambda *s: _rng.normal(s) * 0.05)(B, S, Dm)),
            "w_gate": _w((lambda *s: _rng.normal(s) * 1.6)(Dm, Df) * (Dm ** -0.5)),
            "w_up": _w((lambda *s: _rng.normal(s) * 1.6)(Dm, Df) * (Dm ** -0.5)),
            "w_down": _w((lambda *s: _rng.normal(s) * 1.6)(Df, Dm) * (Df ** -0.5)),
        }
    _B_in = _B_setup()

    return {
        "A_x": _A_in["x"],
        "A_Lambda_re": _A_in["Lambda_re"],
        "A_Lambda_im": _A_in["Lambda_im"],
        "A_B_re": _A_in["B_re"],
        "A_B_im": _A_in["B_im"],
        "A_C_re": _A_in["C_re"],
        "A_C_im": _A_in["C_im"],
        "A_log_dt": _A_in["log_dt"],
        "A_Dskip": _A_in["Dskip"],
        "B_x": _B_in["x"],
        "B_w_gate": _B_in["w_gate"],
        "B_w_up": _B_in["w_up"],
        "B_w_down": _B_in["w_down"],
        "gate_w": _w((lambda *s: _rng.normal(s) * 0.05)(1024) * 16.0),
    }

def reference(A_x, A_Lambda_re, A_Lambda_im, A_B_re, A_B_im, A_C_re, A_C_im, A_log_dt, A_Dskip, B_x, B_w_gate, B_w_up, B_w_down, gate_w):
    def _A_ref(x, Lambda_re, Lambda_im, B_re, B_im, C_re, C_im, log_dt, Dskip):
        Bsz, L, H = x.shape
        Lam = Lambda_re + 1j * Lambda_im
        Bmat = B_re + 1j * B_im
        Cmat = C_re + 1j * C_im
        dt = jnp.exp(log_dt)
        Lam_bar = jnp.exp(dt * Lam)
        B_bar = ((Lam_bar - 1.0) / Lam)[:, None] * Bmat
        Bu = jnp.einsum("bld,pd->blp", x + 0j, B_bar)
        h = jnp.zeros_like(Bu[:, 0, :])
        hs = []
        for t in range(L):
            h = Lam_bar[None, :] * h + Bu[:, t, :]
            hs.append(h)
        hseq = jnp.stack(hs, 1)
        y = 2.0 * jnp.einsum("blp,dp->bld", hseq, Cmat).real + x * Dskip[None, None, :]
        return y

    def _B_ref(x, w_gate, w_up, w_down):
        g = jnp.einsum("bsd,df->bsf", x, w_gate)
        u = jnp.einsum("bsd,df->bsf", x, w_up)
        h = _gelu(g) * u
        return jnp.einsum("bsf,fd->bsd", h, w_down)

    x = A_x
    g = _sigmoid((x * gate_w).sum(-1, keepdims=True))
    a = _A_ref(x, A_Lambda_re, A_Lambda_im, A_B_re, A_B_im, A_C_re, A_C_im, A_log_dt, A_Dskip)
    b = _B_ref(x, B_w_gate, B_w_up, B_w_down)
    return g * a + (1 - g) * b
```

```python
import functools
import math

import jax
import jax.numpy as jnp
import jax.experimental.pallas as pl
import jax.experimental.pallas.tpu as pltpu

_F32 = jnp.float32
_BF16 = jnp.bfloat16
_NT = (((1,), (1,)), ((), ()))


def _gelu_tanh(x):
    c = math.sqrt(2.0 / math.pi)
    return 0.5 * x * (1.0 + jnp.tanh(c * (x + 0.044715 * (x * x * x))))


def _kernel(x_ref, lre_ref, lim_ref, ldt_ref, dskip_ref, gw_ref,
            bre_hbm, bim_hbm, cre_hbm, cim_hbm, wg_hbm, wu_hbm, wd_hbm,
            o_ref,
            bre_ref, bim_ref, cre_ref, cim_ref, wg_ref, wu_ref, wd_ref,
            par_ref, carry_ref, u_ref, h_ref, acc_ref, sems,
            *, tc, p_dim, d_dim, f_dim, fb, fd):
    step = pl.program_id(0)
    P = p_dim
    nf = f_dim // fb
    npiece = tc // 16

    def cp_small(k):
        src, dst = ((bre_hbm, bre_ref), (bim_hbm, bim_ref),
                    (cre_hbm, cre_ref), (cim_hbm, cim_ref))[k]
        return pltpu.make_async_copy(src, dst, sems.at[k])

    nfd = f_dim // fd

    def blk(j, w):
        if isinstance(j, int):
            return pl.ds(j * w, w)
        return pl.ds(pl.multiple_of(j * w, w), w)

    def fslice(j):
        return blk(j, fd)

    def cp_g(j):
        cs = fslice(j)
        return pltpu.make_async_copy(wg_hbm.at[:, cs], wg_ref.at[:, cs], sems.at[4 + 3 * j])

    def cp_u(j):
        cs = fslice(j)
        return pltpu.make_async_copy(wu_hbm.at[:, cs], wu_ref.at[:, cs], sems.at[5 + 3 * j])

    def cp_d(j):
        cs = fslice(j)
        return pltpu.make_async_copy(wd_hbm.at[cs, :], wd_ref.at[cs, :], sems.at[6 + 3 * j])

    def init():
        for k in range(4):
            cp_small(k).start()
        for j in range(nfd):
            cp_g(j).start()
            cp_u(j).start()
            cp_d(j).start()

        lre = lre_ref[...].astype(_F32)
        lim = lim_ref[...].astype(_F32)
        dt = jnp.exp(ldt_ref[...].astype(_F32)).astype(_BF16).astype(_F32)
        mag = jnp.exp(dt * lre)
        ang = dt * lim
        lb_re = mag * jnp.cos(ang)
        lb_im = mag * jnp.sin(ang)
        nre = lb_re - 1.0
        nim = lb_im
        den = lre * lre + lim * lim
        s_re = (nre * lre + nim * lim) / den
        s_im = (nim * lre - nre * lim) / den
        pw_re = [lb_re]
        pw_im = [lb_im]
        for r in range(7):
            q_re, q_im = pw_re[-1], pw_im[-1]
            pw_re.append(q_re * lb_re - q_im * lb_im)
            pw_im.append(q_re * lb_im + q_im * lb_re)
        par_ref[0] = jnp.concatenate(pw_re, axis=0)
        par_ref[1] = jnp.concatenate(pw_im, axis=0)
        sub = jax.lax.broadcasted_iota(jnp.int32, (8, P), 0)
        for k, d in enumerate((1, 2, 4)):
            par_ref[2 + 2 * k] = jnp.where(sub >= d, jnp.broadcast_to(pw_re[d - 1], (8, P)), 0.0)
            par_ref[3 + 2 * k] = jnp.where(sub >= d, jnp.broadcast_to(pw_im[d - 1], (8, P)), 0.0)
        par_ref[8] = jnp.broadcast_to(2.0 * s_re, (8, P))
        par_ref[9] = jnp.broadcast_to(2.0 * s_im, (8, P))
        carry_ref[...] = jnp.zeros(carry_ref.shape, _F32)

    def scan_piece(m, c):
        c_re, c_im = c
        if isinstance(m, int):
            rows = pl.ds(16 * m, 16)
        else:
            rows = pl.ds(pl.multiple_of(16 * m, 16), 16)
        v_re = u_ref[rows, 0:P].reshape(2, 8, P)
        v_im = u_ref[rows, P:2 * P].reshape(2, 8, P)
        for k, d in enumerate((1, 2, 4)):
            m_re = par_ref[2 + 2 * k][None]
            m_im = par_ref[3 + 2 * k][None]
            r_re = pltpu.roll(v_re, d, 1)
            r_im = pltpu.roll(v_im, d, 1)
            v_re, v_im = (v_re + (m_re * r_re - m_im * r_im),
                          v_im + (m_re * r_im + m_im * r_re))
        pw_re = par_ref[0]
        pw_im = par_ref[1]
        s_re = par_ref[8]
        s_im = par_ref[9]
        outs_re = []
        outs_im = []
        for q in range(2):
            cb_re = jnp.broadcast_to(c_re, (8, P))
            cb_im = jnp.broadcast_to(c_im, (8, P))
            h_re = v_re[q] + (pw_re * cb_re - pw_im * cb_im)
            h_im = v_im[q] + (pw_re * cb_im + pw_im * cb_re)
            c_re = h_re[7:8, :]
            c_im = h_im[7:8, :]
            outs_re.append(s_re * h_re - s_im * h_im)
            outs_im.append(-(s_re * h_im + s_im * h_re))
        h_ref[rows, 0:P] = jnp.concatenate(outs_re, axis=0).astype(_BF16)
        h_ref[rows, P:2 * P] = jnp.concatenate(outs_im, axis=0).astype(_BF16)
        return c_re, c_im

    def gate_of(xf):
        gl = jnp.sum(xf * gw_ref[...].astype(_F32), axis=-1, keepdims=True)
        return 1.0 / (1.0 + jnp.exp(-gl))

    def ssm_out(xf):
        a = jax.lax.dot_general(h_ref[:, 0:P], cre_ref[...], _NT, preferred_element_type=_F32)
        a = a + jax.lax.dot_general(h_ref[:, P:2 * P], cim_ref[...], _NT,
                                    preferred_element_type=_F32)
        return a + xf * dskip_ref[...].astype(_F32)

    def first_body():
        xb = x_ref[...]
        nq = P // 256

        def ure(j, carry):
            u_ref[:, blk(j, 256)] = jax.lax.dot_general(
                xb, bre_ref[blk(j, 256), :], _NT, preferred_element_type=_F32)
            return carry

        def uim(j, carry):
            u_ref[:, blk(nq + j, 256)] = jax.lax.dot_general(
                xb, bim_ref[blk(j, 256), :], _NT, preferred_element_type=_F32)
            return carry

        cp_small(0).wait()
        jax.lax.fori_loop(0, nq, ure, 0)
        cp_small(1).wait()
        jax.lax.fori_loop(0, nq, uim, 0)
        c = jax.lax.fori_loop(0, npiece, scan_piece, (carry_ref[0:1, :], carry_ref[1:2, :]))
        carry_ref[0:1, :] = c[0]
        carry_ref[1:2, :] = c[1]
        cp_small(2).wait()
        cp_small(3).wait()

        def yproj(j, carry):
            cs = blk(j, 256)
            a = jax.lax.dot_general(h_ref[:, 0:P], cre_ref[cs, :], _NT,
                                    preferred_element_type=_F32)
            a = a + jax.lax.dot_general(h_ref[:, P:2 * P], cim_ref[cs, :], _NT,
                                        preferred_element_type=_F32)
            acc_ref[:, cs] = a + x_ref[:, cs].astype(_F32) * dskip_ref[:, cs].astype(_F32)
            return carry

        jax.lax.fori_loop(0, d_dim // 256, yproj, 0)
        o_ref[...] = jnp.zeros(o_ref.shape, _F32)

        def ffn(j, carry):
            cs = fslice(j)
            cp_g(j).wait()
            cp_u(j).wait()
            g = jnp.dot(xb, wg_ref[:, cs], preferred_element_type=_F32)
            u = jnp.dot(xb, wu_ref[:, cs], preferred_element_type=_F32)
            hh = (_gelu_tanh(g) * u).astype(_BF16)
            cp_d(j).wait()
            o_ref[...] += jnp.dot(hh, wd_ref[cs, :], preferred_element_type=_F32)
            return carry

        jax.lax.fori_loop(0, nfd, ffn, 0)
        gate = gate_of(xb.astype(_F32))
        o_ref[...] = gate * acc_ref[...] + (1.0 - gate) * o_ref[...]

    def body():
        xb = x_ref[...]
        xf = xb.astype(_F32)
        gate = gate_of(xf)

        u_ref[:, 0:P] = jax.lax.dot_general(xb, bre_ref[...], _NT, preferred_element_type=_F32)
        u_ref[:, P:2 * P] = jax.lax.dot_general(xb, bim_ref[...], _NT, preferred_element_type=_F32)

        c = (carry_ref[0:1, :], carry_ref[1:2, :])
        done = 0

        acc = jnp.zeros((tc, d_dim), _F32)
        for j in range(nf):
            cs = blk(j, fb)
            g = jnp.dot(xb, wg_ref[:, cs], preferred_element_type=_F32)
            u = jnp.dot(xb, wu_ref[:, cs], preferred_element_type=_F32)
            tgt = min(npiece, ((j + 1) * npiece + nf - 2) // (nf - 1))
            while done < tgt:
                c = scan_piece(done, c)
                done += 1
            hh = (_gelu_tanh(g) * u).astype(_BF16)
            acc = acc + jnp.dot(hh, wd_ref[cs, :], preferred_element_type=_F32)
        carry_ref[0:1, :] = c[0]
        carry_ref[1:2, :] = c[1]

        o_ref[...] = gate * ssm_out(xf) + (1.0 - gate) * acc

    @pl.when(step == 0)
    def _():
        init()
        first_body()

    @pl.when(step > 0)
    def _():
        body()


@jax.jit
def pallas_gated_mix__ssm_conv_s5__glu_gated_geglu__prompt_kernel(
    A_x: jax.Array,
    A_Lambda_re: jax.Array,
    A_Lambda_im: jax.Array,
    A_B_re: jax.Array,
    A_B_im: jax.Array,
    A_C_re: jax.Array,
    A_C_im: jax.Array,
    A_log_dt: jax.Array,
    A_Dskip: jax.Array,
    B_x: jax.Array,
    B_w_gate: jax.Array,
    B_w_up: jax.Array,
    B_w_down: jax.Array,
    gate_w: jax.Array,
):
    Bsz, L, D = A_x.shape
    assert Bsz == 1
    P = A_B_re.shape[0]
    F = B_w_gate.shape[1]
    tc = 256
    fb = 512
    fd = 256
    nt = L // tc

    x2 = A_x.reshape(L, D)
    row = lambda v: v.reshape(1, -1)

    const = lambda shape: pl.BlockSpec(shape, lambda i: (0, 0),
                                       pipeline_mode=pl.Buffered(1))
    hbm = pl.BlockSpec(memory_space=pl.ANY)
    kern = functools.partial(_kernel, tc=tc, p_dim=P, d_dim=D, f_dim=F, fb=fb, fd=fd)
    out = pl.pallas_call(
        kern,
        grid=(nt,),
        in_specs=[
            pl.BlockSpec((tc, D), lambda i: (i, 0)),
            const((1, P)), const((1, P)), const((1, P)), const((1, D)), const((1, D)),
            hbm, hbm, hbm, hbm, hbm, hbm, hbm,
        ],
        out_specs=pl.BlockSpec((tc, D), lambda i: (i, 0)),
        out_shape=jax.ShapeDtypeStruct((L, D), _F32),
        scratch_shapes=[
            pltpu.VMEM((P, D), _BF16),
            pltpu.VMEM((P, D), _BF16),
            pltpu.VMEM((D, P), _BF16),
            pltpu.VMEM((D, P), _BF16),
            pltpu.VMEM((D, F), _BF16),
            pltpu.VMEM((D, F), _BF16),
            pltpu.VMEM((F, D), _BF16),
            pltpu.VMEM((10, 8, P), _F32),
            pltpu.VMEM((2, P), _F32),
            pltpu.VMEM((tc, 2 * P), _F32),
            pltpu.VMEM((tc, 2 * P), _BF16),
            pltpu.VMEM((tc, D), _F32),
            pltpu.SemaphoreType.DMA((4 + 3 * (F // fd),)),
        ],
        compiler_params=pltpu.CompilerParams(
            dimension_semantics=("arbitrary",),
            vmem_limit_bytes=100 * 1024 * 1024,
        ),
    )(x2, row(A_Lambda_re), row(A_Lambda_im), row(A_log_dt), row(A_Dskip),
      row(gate_w), A_B_re, A_B_im, A_C_re, A_C_im, B_w_gate, B_w_up, B_w_down)
    return out.reshape(Bsz, L, D)
```

```python
import functools
import math

import jax
import jax.numpy as jnp
import jax.experimental.pallas as pl
import jax.experimental.pallas.tpu as pltpu

_F32 = jnp.float32
_BF16 = jnp.bfloat16
_NT = (((1,), (1,)), ((), ()))


def _gelu_tanh(x):
    c = math.sqrt(2.0 / math.pi)
    return 0.5 * x * (1.0 + jnp.tanh(c * (x + 0.044715 * (x * x * x))))


def _kernel(x_ref, lre_ref, lim_ref, ldt_ref, dskip_ref, gw_ref,
            bre_hbm, bim_hbm, cre_hbm, cim_hbm, wg_hbm, wu_hbm, wd_hbm,
            o_ref,
            bre_ref, bim_ref, cre_ref, cim_ref, wg_ref, wu_ref, wd_ref,
            par_ref, carry_ref, vec_ref, u_ref, h_ref, acc_ref, sems,
            *, tc, p_dim, d_dim, f_dim, fb, fd):
    step = pl.program_id(0)
    P = p_dim
    nf = f_dim // fb
    npiece = tc // 16

    def cp_small(k):
        src, dst = ((bre_hbm, bre_ref), (bim_hbm, bim_ref),
                    (cre_hbm, cre_ref), (cim_hbm, cim_ref))[k]
        return pltpu.make_async_copy(src, dst, sems.at[k])

    nfd = f_dim // fd

    def blk(j, w):
        if isinstance(j, int):
            return pl.ds(j * w, w)
        return pl.ds(pl.multiple_of(j * w, w), w)

    def fslice(j):
        return blk(j, fd)

    def cp_g(j):
        cs = fslice(j)
        return pltpu.make_async_copy(wg_hbm.at[:, cs], wg_ref.at[:, cs], sems.at[4 + 3 * j])

    def cp_u(j):
        cs = fslice(j)
        return pltpu.make_async_copy(wu_hbm.at[:, cs], wu_ref.at[:, cs], sems.at[5 + 3 * j])

    def cp_d(j):
        cs = fslice(j)
        return pltpu.make_async_copy(wd_hbm.at[cs, :], wd_ref.at[cs, :], sems.at[6 + 3 * j])

    def init():
        for k in range(4):
            cp_small(k).start()
        for j in range(nfd):
            cp_g(j).start()
            cp_u(j).start()
            cp_d(j).start()

        lre = lre_ref[...].astype(_F32).reshape(1, P)
        lim = lim_ref[...].astype(_F32).reshape(1, P)
        dt = jnp.exp(ldt_ref[...].astype(_F32).reshape(1, P)).astype(_BF16).astype(_F32)
        mag = jnp.exp(dt * lre)
        ang = dt * lim
        lb_re = mag * jnp.cos(ang)
        lb_im = mag * jnp.sin(ang)
        nre = lb_re - 1.0
        nim = lb_im
        den = lre * lre + lim * lim
        s_re = (nre * lre + nim * lim) / den
        s_im = (nim * lre - nre * lim) / den
        pw_re = [lb_re]
        pw_im = [lb_im]
        for r in range(7):
            q_re, q_im = pw_re[-1], pw_im[-1]
            pw_re.append(q_re * lb_re - q_im * lb_im)
            pw_im.append(q_re * lb_im + q_im * lb_re)
        par_ref[0] = jnp.concatenate(pw_re, axis=0)
        par_ref[1] = jnp.concatenate(pw_im, axis=0)
        sub = jax.lax.broadcasted_iota(jnp.int32, (8, P), 0)
        for k, d in enumerate((1, 2, 4)):
            par_ref[2 + 2 * k] = jnp.where(sub >= d, jnp.broadcast_to(pw_re[d - 1], (8, P)), 0.0)
            par_ref[3 + 2 * k] = jnp.where(sub >= d, jnp.broadcast_to(pw_im[d - 1], (8, P)), 0.0)
        par_ref[8] = jnp.broadcast_to(2.0 * s_re, (8, P))
        par_ref[9] = jnp.broadcast_to(2.0 * s_im, (8, P))
        carry_ref[...] = jnp.zeros(carry_ref.shape, _F32)
        vec_ref[0:1, :] = dskip_ref[...].astype(_F32).reshape(1, d_dim)
        vec_ref[1:2, :] = gw_ref[...].astype(_F32).reshape(1, d_dim)

    def scan_piece(m, c):
        c_re, c_im = c
        if isinstance(m, int):
            rows = pl.ds(16 * m, 16)
        else:
            rows = pl.ds(pl.multiple_of(16 * m, 16), 16)
        v_re = u_ref[rows, 0:P].reshape(2, 8, P)
        v_im = u_ref[rows, P:2 * P].reshape(2, 8, P)
        for k, d in enumerate((1, 2, 4)):
            m_re = par_ref[2 + 2 * k][None]
            m_im = par_ref[3 + 2 * k][None]
            r_re = pltpu.roll(v_re, d, 1)
            r_im = pltpu.roll(v_im, d, 1)
            v_re, v_im = (v_re + (m_re * r_re - m_im * r_im),
                          v_im + (m_re * r_im + m_im * r_re))
        pw_re = par_ref[0]
        pw_im = par_ref[1]
        s_re = par_ref[8]
        s_im = par_ref[9]
        outs_re = []
        outs_im = []
        for q in range(2):
            cb_re = jnp.broadcast_to(c_re, (8, P))
            cb_im = jnp.broadcast_to(c_im, (8, P))
            h_re = v_re[q] + (pw_re * cb_re - pw_im * cb_im)
            h_im = v_im[q] + (pw_re * cb_im + pw_im * cb_re)
            c_re = h_re[7:8, :]
            c_im = h_im[7:8, :]
            outs_re.append(s_re * h_re - s_im * h_im)
            outs_im.append(-(s_re * h_im + s_im * h_re))
        h_ref[rows, 0:P] = jnp.concatenate(outs_re, axis=0).astype(_BF16)
        h_ref[rows, P:2 * P] = jnp.concatenate(outs_im, axis=0).astype(_BF16)
        return c_re, c_im

    def gate_of(xf):
        gl = jnp.sum(xf * vec_ref[1:2, :], axis=-1, keepdims=True)
        return 1.0 / (1.0 + jnp.exp(-gl))

    def ssm_out(xf):
        a = jax.lax.dot_general(h_ref[:, 0:P], cre_ref[...], _NT, preferred_element_type=_F32)
        a = a + jax.lax.dot_general(h_ref[:, P:2 * P], cim_ref[...], _NT,
                                    preferred_element_type=_F32)
        return a + xf * vec_ref[0:1, :]

    def first_body():
        xb = x_ref[...]
        nq = P // 256

        def ure(j, carry):
            u_ref[:, blk(j, 256)] = jax.lax.dot_general(
                xb, bre_ref[blk(j, 256), :], _NT, preferred_element_type=_F32)
            return carry

        def uim(j, carry):
            u_ref[:, blk(nq + j, 256)] = jax.lax.dot_general(
                xb, bim_ref[blk(j, 256), :], _NT, preferred_element_type=_F32)
            return carry

        cp_small(0).wait()
        jax.lax.fori_loop(0, nq, ure, 0)
        cp_small(1).wait()
        jax.lax.fori_loop(0, nq, uim, 0)
        c = jax.lax.fori_loop(0, npiece, scan_piece, (carry_ref[0:1, :], carry_ref[1:2, :]))
        carry_ref[0:1, :] = c[0]
        carry_ref[1:2, :] = c[1]
        cp_small(2).wait()
        cp_small(3).wait()

        def yproj(j, carry):
            cs = blk(j, 256)
            a = jax.lax.dot_general(h_ref[:, 0:P], cre_ref[cs, :], _NT,
                                    preferred_element_type=_F32)
            a = a + jax.lax.dot_general(h_ref[:, P:2 * P], cim_ref[cs, :], _NT,
                                        preferred_element_type=_F32)
            acc_ref[:, cs] = a + x_ref[:, cs].astype(_F32) * vec_ref[0:1, cs]
            return carry

        jax.lax.fori_loop(0, d_dim // 256, yproj, 0)
        o_ref[...] = jnp.zeros(o_ref.shape, _F32)

        def ffn(j, carry):
            cs = fslice(j)
            cp_g(j).wait()
            cp_u(j).wait()
            g = jnp.dot(xb, wg_ref[:, cs], preferred_element_type=_F32)
            u = jnp.dot(xb, wu_ref[:, cs], preferred_element_type=_F32)
            hh = (_gelu_tanh(g) * u).astype(_BF16)
            cp_d(j).wait()
            o_ref[...] += jnp.dot(hh, wd_ref[cs, :], preferred_element_type=_F32)
            return carry

        jax.lax.fori_loop(0, nfd, ffn, 0)
        gate = gate_of(xb.astype(_F32))
        o_ref[...] = gate * acc_ref[...] + (1.0 - gate) * o_ref[...]

    def body():
        xb = x_ref[...]
        xf = xb.astype(_F32)
        gate = gate_of(xf)

        c = (carry_ref[0:1, :], carry_ref[1:2, :])
        NS = 4
        rs = tc // NS
        when = [(q * (nf - 1)) // NS for q in range(NS)]

        acc = jnp.zeros((tc, d_dim), _F32)
        for j in range(nf):
            cs = blk(j, fb)
            for q in range(NS):
                if when[q] == j:
                    r = pl.ds(q * rs, rs)
                    u_ref[r, 0:P] = jax.lax.dot_general(
                        x_ref[r, :], bre_ref[...], _NT, preferred_element_type=_F32)
                    u_ref[r, P:2 * P] = jax.lax.dot_general(
                        x_ref[r, :], bim_ref[...], _NT, preferred_element_type=_F32)
            g = jnp.dot(xb, wg_ref[:, cs], preferred_element_type=_F32)
            u = jnp.dot(xb, wu_ref[:, cs], preferred_element_type=_F32)
            for q in range(NS):
                if when[q] == j:
                    for m in range(q * rs // 16, (q + 1) * rs // 16):
                        c = scan_piece(m, c)
            hh = (_gelu_tanh(g) * u).astype(_BF16)
            acc = acc + jnp.dot(hh, wd_ref[cs, :], preferred_element_type=_F32)
        carry_ref[0:1, :] = c[0]
        carry_ref[1:2, :] = c[1]

        o_ref[...] = gate * ssm_out(xf) + (1.0 - gate) * acc

    @pl.when(step == 0)
    def _():
        init()
        first_body()

    @pl.when(step > 0)
    def _():
        body()


@jax.jit
def pallas_gated_mix__ssm_conv_s5__glu_gated_geglu__prompt_kernel(
    A_x: jax.Array,
    A_Lambda_re: jax.Array,
    A_Lambda_im: jax.Array,
    A_B_re: jax.Array,
    A_B_im: jax.Array,
    A_C_re: jax.Array,
    A_C_im: jax.Array,
    A_log_dt: jax.Array,
    A_Dskip: jax.Array,
    B_x: jax.Array,
    B_w_gate: jax.Array,
    B_w_up: jax.Array,
    B_w_down: jax.Array,
    gate_w: jax.Array,
):
    Bsz, L, D = A_x.shape
    assert Bsz == 1
    P = A_B_re.shape[0]
    F = B_w_gate.shape[1]
    tc = 256
    fb = 512
    fd = 256
    nt = L // tc

    x2 = A_x.reshape(L, D)

    const = lambda n: pl.BlockSpec((n,), lambda i: (0,), pipeline_mode=pl.Buffered(1))
    hbm = pl.BlockSpec(memory_space=pl.ANY)
    kern = functools.partial(_kernel, tc=tc, p_dim=P, d_dim=D, f_dim=F, fb=fb, fd=fd)
    out = pl.pallas_call(
        kern,
        grid=(nt,),
        in_specs=[
            pl.BlockSpec((tc, D), lambda i: (i, 0)),
            const(P), const(P), const(P), const(D), const(D),
            hbm, hbm, hbm, hbm, hbm, hbm, hbm,
        ],
        out_specs=pl.BlockSpec((tc, D), lambda i: (i, 0)),
        out_shape=jax.ShapeDtypeStruct((L, D), _F32),
        scratch_shapes=[
            pltpu.VMEM((P, D), _BF16),
            pltpu.VMEM((P, D), _BF16),
            pltpu.VMEM((D, P), _BF16),
            pltpu.VMEM((D, P), _BF16),
            pltpu.VMEM((D, F), _BF16),
            pltpu.VMEM((D, F), _BF16),
            pltpu.VMEM((F, D), _BF16),
            pltpu.VMEM((10, 8, P), _F32),
            pltpu.VMEM((2, P), _F32),
            pltpu.VMEM((2, D), _F32),
            pltpu.VMEM((tc, 2 * P), _F32),
            pltpu.VMEM((tc, 2 * P), _BF16),
            pltpu.VMEM((tc, D), _F32),
            pltpu.SemaphoreType.DMA((4 + 3 * (F // fd),)),
        ],
        compiler_params=pltpu.CompilerParams(
            dimension_semantics=("arbitrary",),
            vmem_limit_bytes=100 * 1024 * 1024,
        ),
    )(x2, A_Lambda_re, A_Lambda_im, A_log_dt, A_Dskip,
      gate_w, A_B_re, A_B_im, A_C_re, A_C_im, B_w_gate, B_w_up, B_w_down)
    return out.reshape(Bsz, L, D)
```
